```python
import os as _os
_os.environ.setdefault("JAX_PLATFORMS", "cpu")
import jax
import jax.numpy as jnp

def _softmax(x, axis=-1):
    return jax.nn.softmax(x, axis=axis)
def _gelu(x):
    return jax.nn.gelu(x, approximate=True)
def _silu(x):
    return jax.nn.silu(x)
def _sigmoid(x):
    return jax.nn.sigmoid(x)
def _layernorm(x, axis=-1, eps=1e-5):
    m = jnp.mean(x, axis=axis, keepdims=True)
    v = jnp.var(x, axis=axis, keepdims=True)
    return (x - m) / jnp.sqrt(v + eps)
def _scatter_add(tgt, idx, src, axis=0):
    return tgt.at[idx].add(src)
def _segment_sum(src, seg, n):
    return jax.ops.segment_sum(src, seg, n)
class _Rng:
    def __init__(self, key):
        self._k = key
    def _next(self):
        self._k, sub = jax.random.split(self._k)
        return sub
    def normal(self, shape):
        return jax.random.normal(self._next(), shape, dtype=jnp.bfloat16)
    def randint(self, lo, hi, shape):
        return jax.random.randint(self._next(), shape, lo, hi, dtype=jnp.int32)
    def uniform(self, shape, lo=0.0, hi=1.0):
        return jax.random.uniform(self._next(), shape, jnp.bfloat16, lo, hi)
    def permutation(self, n):
        return jax.random.permutation(self._next(), n)


kernel_name = 'concat_heads__grouped_kv_mqa__sliding_block__prompt'

def setup_inputs():
    _rng = _Rng(jax.random.key(int.from_bytes(__import__("os").urandom(4), "little")))
    _w = (lambda a: (lambda t: t.astype(jnp.bfloat16) if jnp.issubdtype(t.dtype, jnp.floating) else t)(jnp.asarray(a)))
    def _A_setup():
        B, S, D, H = 1, 2048, 1024, 32
        Dh = D // H
        return {
            "x": _w((lambda *s: _rng.normal(s) * 0.05)(B, S, D)),
            "wq": _w((lambda *s: _rng.normal(s) * 1.6)(D, H * Dh)),
            "wk": _w((lambda *s: _rng.normal(s) * 1.6)(D, Dh)),
            "wv": _w((lambda *s: _rng.normal(s) * 0.1)(D, Dh)),
            "wo": _w((lambda *s: _rng.normal(s) * 0.1)(H * Dh, D)),
        }
    _A_in = _A_setup()

    def _B_setup():
        B, S, D = 1, 2048, 1024
        return {
            "x": _w((lambda *s: _rng.normal(s) * 0.2)(B, S, D)),
            "wqkv": _w((lambda *s: _rng.normal(s) * 0.2)(D, 3 * D)),
            "wo": _w((lambda *s: _rng.normal(s) * 0.05)(D, D)),
        }
    _B_in = _B_setup()

    return {
        "A_x": _A_in["x"],
        "A_wq": _A_in["wq"],
        "A_wk": _A_in["wk"],
        "A_wv": _A_in["wv"],
        "A_wo": _A_in["wo"],
        "B_x": _B_in["x"],
        "B_wqkv": _B_in["wqkv"],
        "B_wo": _B_in["wo"],
    }

def reference(A_x, A_wq, A_wk, A_wv, A_wo, B_x, B_wqkv, B_wo):
    def _A_ref(x, wq, wk, wv, wo):
        B, S, D = x.shape
        H = 32
        Dh = D // H
        q = (lambda x, *d: x.transpose(*d))((x @ wq).reshape(B, S, H, Dh), 0, 2, 1, 3)
        k = x @ wk
        v = x @ wv
        scores = jnp.einsum("bhqd,bkd->bhqk", q, k) * (Dh ** -0.5)
        p = _softmax(scores, axis=-1)
        o = jnp.einsum("bhqk,bkd->bhqd", p, v)
        return (lambda x, *d: x.transpose(*d))(o, 0, 2, 1, 3).reshape(B, S, H * Dh) @ wo

    def _B_ref(x, wqkv, wo):
        B, S, D = x.shape
        H = 32; Dh = D // H; W = 256
        qkv = (lambda x, *d: x.transpose(*d))((x @ wqkv).reshape(B, S, 3, H, Dh), 2, 0, 3, 1, 4)
        q, k, v = qkv[0], qkv[1], qkv[2]
        scores = jnp.einsum("bhqd,bhkd->bhqk", q, k) * (Dh ** -0.5)
        idx = jnp.arange(S)
        mask = (idx[:, None] - idx[None, :] >= 0) & (idx[:, None] - idx[None, :] < W)
        scores = jnp.where(mask[None, None], scores, -1e9)
        p = _softmax(scores, axis=-1)
        o = jnp.einsum("bhqk,bhkd->bhqd", p, v)
        return (lambda x, *d: x.transpose(*d))(o, 0, 2, 1, 3).reshape(B, S, D) @ wo

    a = _A_ref(A_x, A_wq, A_wk, A_wv, A_wo)
    b = _B_ref(B_x, B_wqkv, B_wo)
    return jnp.concatenate([a, b], axis=-1)
```

```python
import math

import jax
import jax.numpy as jnp
from jax import lax
import jax.experimental.pallas as pl
import jax.experimental.pallas.tpu as pltpu

SEQ = 2048
DM = 1024
DH = 32
NH = 32
WIN = 256

BF = jnp.bfloat16
F32 = jnp.float32
U32 = jnp.uint32

LOG2E = 1.4426950408889634
QSCALE = (DH ** -0.5) * LOG2E
L_LO = 2.0 ** -80
L_HI = 2.0 ** 100
O_MAX = 3.0e38

NT_DIMS = (((1,), (1,)), ((), ()))

HPU = 8
CH = 256
QB = 512


def _pk(x):
    return pltpu.bitcast(x, U32)


def _upk(x):
    return pltpu.bitcast(x, BF)


def _flag_unsafe(bad, l, o):
    ok_l = jnp.logical_and(l >= L_LO, l <= L_HI)
    n = l.shape[1] // 128
    for j in range(n):
        bad = jnp.where(ok_l[:, j * 128:(j + 1) * 128], bad, 1.0)
    rows = o.shape[0] // 8
    ok_o = jnp.abs(o) <= O_MAX
    for r in range(rows):
        for j in range(n):
            bad = jnp.where(ok_o[r * 8:(r + 1) * 8, j * 128:(j + 1) * 128], bad, 1.0)
    return bad


def _kernel(ax_h, awq_h, awk_h, awv_h, awo_h, bx_h, bwqkv_h, bwo_h, out_h,
            ax, awq, awk, awv, awo, bx, bwqkv, bwo,
            wta, qta, ka, vta, oa, pa, accs, ls,
            wtb, qtb, kb, vtb, ob, pb, accb, lb,
            stage, isem, osem):
    nqb = SEQ // QB

    def xcopy(src, dst, qb, sem):
        return pltpu.make_async_copy(src.at[pl.ds(qb * QB, QB), :],
                                     dst.at[pl.ds(qb * QB, QB), :], sem)

    cp_awq = pltpu.make_async_copy(awq_h, awq, isem.at[0])
    cp_awk = pltpu.make_async_copy(awk_h, awk, isem.at[1])
    cp_awv = pltpu.make_async_copy(awv_h, awv, isem.at[2])
    cp_awo = pltpu.make_async_copy(awo_h, awo, isem.at[3])
    cp_bw = pltpu.make_async_copy(bwqkv_h, bwqkv, isem.at[4])
    cp_bwo = pltpu.make_async_copy(bwo_h, bwo, isem.at[5])
    cp_ax = [xcopy(ax_h, ax, i, isem.at[6 + i]) for i in range(nqb)]
    cp_bx = [xcopy(bx_h, bx, i, isem.at[6 + nqb + i]) for i in range(nqb)]

    cp_awq.start()
    cp_awv.start()
    cp_awk.start()
    cp_ax[0].start()
    for c in cp_ax[1:]:
        c.start()
    cp_bw.start()
    cp_awo.start()
    for c in cp_bx:
        c.start()
    cp_bwo.start()

    cp_awq.wait()
    for b in range(DM // 128):
        wta[b * 128:(b + 1) * 128, :] = awq[:, b * 128:(b + 1) * 128].T
    cp_awv.wait()
    wta[DM:DM + DH, :] = awv[...].T
    cp_awk.wait()
    wta[DM + DH:DM + 2 * DH, :] = awk[...].T
    for qb in range(nqb):
        cp_ax[qb].wait()
        res = lax.dot_general(wta[...], ax[qb * QB:(qb + 1) * QB, :], NT_DIMS,
                              preferred_element_type=F32)
        qs = slice(qb * QB, (qb + 1) * QB)
        qta[:, qs] = _pk((res[:DM] * QSCALE).astype(BF))
        vta[:, qs] = _pk(res[DM:DM + DH].astype(BF))
        ka[qb * QB // 2:(qb + 1) * QB // 2, :] = _pk(res[DM + DH:].T.astype(BF))

    na = HPU * 128
    noct = NH // HPU
    ncha = SEQ // CH

    def a_finalize(acc, l, u, bad):
        t = u // noct
        oc = u % noct
        lt = jnp.sum(l, axis=0, keepdims=True)
        o = acc * (1.0 / lt)
        bad = _flag_unsafe(bad, jnp.broadcast_to(lt, (8, na)), o)
        for g in range(HPU // 4):
            st = jnp.concatenate([o[:, (4 * g + j) * 128:(4 * g + j + 1) * 128] for j in range(4)],
                                 axis=0)
            col = pl.multiple_of(oc * (HPU * DH) + g * 128, 128)
            oa[pl.ds(pl.multiple_of(t * 128, 128), 128), pl.ds(col, 128)] = st.T.astype(BF)
        return bad

    def a_qt(u):
        t = u // noct
        oc = u % noct
        qall = qta[pl.ds(pl.multiple_of(oc * (HPU * DH // 2), HPU * DH // 2), HPU * DH // 2),
                   pl.ds(pl.multiple_of(t * 128, 128), 128)]
        return jnp.concatenate([_upk(qall[j * (DH // 2):(j + 1) * (DH // 2)]) for j in range(HPU)],
                               axis=1)

    def a_body(u, bad):
        qt = a_qt(u)
        l = jnp.zeros((8, na), F32)
        acc = jnp.zeros((DH, na), F32)
        bad = a_finalize(accs[...], ls[...], jnp.maximum(u - 1, 0), bad)
        for c in range(ncha + 1):
            if c < ncha:
                kc = _upk(ka[c * CH // 2:(c + 1) * CH // 2, :])
                p = jnp.exp2(jnp.dot(kc, qt, preferred_element_type=F32))
                l = l + p.reshape(CH // 8, 8, na).sum(axis=0)
                pa[c] = _pk(p.astype(BF))
            if c >= 1:
                vc = _upk(vta[:, (c - 1) * CH:c * CH])
                acc = acc + jnp.dot(vc, _upk(pa[c - 1]), preferred_element_type=F32)
        accs[...] = acc
        ls[...] = l
        return bad

    accs[...] = jnp.zeros((DH, na), F32)
    ls[...] = jnp.ones((8, na), F32)
    nunits = (SEQ // 128) * noct
    bad_a = lax.fori_loop(0, nunits, a_body, jnp.zeros((8, 128), F32))
    bad_a = a_finalize(accs[...], ls[...], nunits - 1, bad_a)

    @pl.when(jnp.max(bad_a) > 0.0)
    def _a_fallback():
        def unit(u, _):
            qt = a_qt(u)

            def scores(c):
                kc = _upk(ka[pl.ds(pl.multiple_of(c * 64, 64), 64), :])
                return jnp.dot(kc, qt, preferred_element_type=F32).reshape(16, 8, na)

            def pass1(c, m):
                return jnp.maximum(m, scores(c).max(axis=0))

            m = lax.fori_loop(0, SEQ // 128, pass1, jnp.full((8, na), -jnp.inf, F32))
            m = jnp.broadcast_to(jnp.max(m, axis=0, keepdims=True), (8, na))

            def pass2(c, carry):
                l, acc = carry
                p = jnp.exp2(scores(c) - m[None])
                vc = _upk(vta[:, pl.ds(pl.multiple_of(c * 128, 128), 128)])
                acc = acc + jnp.dot(vc, p.reshape(128, na).astype(BF), preferred_element_type=F32)
                return l + p.sum(axis=0), acc

            l, acc = lax.fori_loop(0, SEQ // 128, pass2,
                                   (jnp.zeros((8, na), F32), jnp.zeros((DH, na), F32)))
            a_finalize(acc, l, u, jnp.zeros((8, 128), F32))
            return 0

        lax.fori_loop(0, nunits, unit, 0)

    cp_awo.wait()
    cp_bw.wait()
    out_copies = []
    for qb in range(nqb):
        qs = slice(qb * QB, (qb + 1) * QB)
        res = jnp.dot(oa[qs, :], awo[...], preferred_element_type=F32)
        stage[0, qs, :] = res.astype(BF)
        cp = pltpu.make_async_copy(stage.at[0, pl.ds(qb * QB, QB), :],
                                   out_h.at[pl.ds(qb * QB, QB), pl.ds(0, DM)], osem.at[qb])
        cp.start()
        out_copies.append(cp)

    for b in range(DM // 128):
        wtb[b * 128:(b + 1) * 128, :] = bwqkv[:, b * 128:(b + 1) * 128].T
        wtb[DM + b * 128:DM + (b + 1) * 128, :] = bwqkv[:, 2 * DM + b * 128:2 * DM + (b + 1) * 128].T
    for qb in range(nqb):
        cp_bx[qb].wait()
        xq = bx[qb * QB:(qb + 1) * QB, :]
        qs = slice(qb * QB, (qb + 1) * QB)
        res = lax.dot_general(wtb[...], xq, NT_DIMS, preferred_element_type=F32)
        qtb[:, qs] = _pk((res[:DM] * QSCALE).astype(BF))
        vtb[:, qs] = _pk(res[DM:].astype(BF))
        kres = jnp.dot(xq, bwqkv[:, DM:2 * DM], preferred_element_type=F32)
        kpk = _pk(kres.astype(BF))
        for g in range(NH // 4):
            kb[g, qb * QB // 2:(qb + 1) * QB // 2, :] = kpk[:, g * 128:(g + 1) * 128]

    nt = SEQ // 128
    row = lax.broadcasted_iota(jnp.int32, (128, 128), 0)
    colq = lax.broadcasted_iota(jnp.int32, (128, 128), 1)

    def tile4(m):
        return jnp.concatenate([m, m, m, m], axis=1)

    def b_weights(g, t):
        q4 = qtb[pl.ds(pl.multiple_of(g * 64, 64), 64), pl.ds(t * 128, 128)]
        z = jnp.zeros((16, 128), U32)
        cols = []
        for j in range(4):
            cols.append(jnp.concatenate(
                [q4[j * 16:(j + 1) * 16] if i == j else z for i in range(4)], axis=0))
        return _upk(jnp.concatenate(cols, axis=1))

    def b_finalize(acc, l, g, t, bad):
        lt = jnp.sum(l, axis=0, keepdims=True)
        o = acc * (1.0 / lt)
        bad = _flag_unsafe(bad, jnp.broadcast_to(lt, (8, 512)), o)
        st = jnp.concatenate([o[:, j * 128:(j + 1) * 128] for j in range(4)], axis=0)
        ob[pl.ds(t * 128, 128), pl.ds(pl.multiple_of(g * 128, 128), 128)] = st.T.astype(BF)
        return bad

    def b_body(g, bad):
        causal = tile4(row <= colq)
        inwin = tile4(row > colq)
        v0 = pl.multiple_of(g * 64, 64)

        def qk(t):
            c0 = max(t - 2, 0)
            nrow = (t + 1 - c0) * 128
            w = b_weights(g, t)
            kc = _upk(kb[g, c0 * 64:c0 * 64 + nrow // 2, :])
            p = jnp.exp2(jnp.dot(kc, w, preferred_element_type=F32))
            parts = []
            for c in range(c0, t + 1):
                pc = p[(c - c0) * 128:(c - c0 + 1) * 128]
                if c == t:
                    pc = jnp.where(causal, pc, 0.0)
                elif c == t - 2:
                    pc = jnp.where(inwin, pc, 0.0)
                parts.append(pc)
            p = jnp.concatenate(parts, axis=0) if len(parts) > 1 else parts[0]
            l = p.reshape(nrow // 8, 8, 512).sum(axis=0)
            pb[t % 2, 0:nrow // 2, :] = _pk(p.astype(BF))
            return l

        def pv(t):
            c0 = max(t - 2, 0)
            nrow = (t + 1 - c0) * 128
            outs = []
            for j in range(4):
                vj = _upk(vtb[pl.ds(v0 + j * 16, 16), c0 * 128:c0 * 128 + nrow])
                pj = _upk(pb[t % 2, 0:nrow // 2, j * 128:(j + 1) * 128])
                outs.append(jnp.dot(vj, pj, preferred_element_type=F32))
            return jnp.concatenate(outs, axis=1)

        bad = b_finalize(accb[...], lb[...], jnp.maximum(g - 1, 0), nt - 1, bad)
        l_prev = None
        acc_prev = None
        l_pp = None
        for t in range(nt + 1):
            l_cur = qk(t) if t < nt else None
            if t >= 2:
                bad = b_finalize(acc_prev, l_pp, g, t - 2, bad)
            if t >= 1:
                acc_prev = pv(t - 1)
                l_pp = l_prev
            l_prev = l_cur
        accb[...] = acc_prev
        lb[...] = l_pp
        return bad

    accb[...] = jnp.zeros((DH, 512), F32)
    lb[...] = jnp.ones((8, 512), F32)
    bad_b = lax.fori_loop(0, NH // 4, b_body, jnp.zeros((8, 128), F32))
    bad_b = b_finalize(accb[...], lb[...], NH // 4 - 1, nt - 1, bad_b)

    @pl.when(jnp.max(bad_b) > 0.0)
    def _b_fallback():
        fill = float(jnp.asarray(-1e9, BF).astype(F32)) if False else -999292928.0 * LOG2E

        def unit(u, _):
            g = u // nt
            t = u % nt
            q4 = qtb[pl.ds(pl.multiple_of(g * 64, 64), 64), pl.ds(pl.multiple_of(t * 128, 128), 128)]
            z = jnp.zeros((16, 128), U32)
            w = _upk(jnp.concatenate(
                [jnp.concatenate([q4[j * 16:(j + 1) * 16] if i == j else z for i in range(4)], axis=0)
                 for j in range(4)], axis=1))

            def scores(c):
                kc = _upk(kb[g, pl.ds(pl.multiple_of(c * 64, 64), 64), :])
                s = jnp.dot(kc, w, preferred_element_type=F32)
                d = (colq + t * 128) - (row + c * 128)
                valid = tile4(jnp.logical_and(d >= 0, d < WIN))
                return jnp.where(valid, s, fill).reshape(16, 8, 512)

            def pass1(c, m):
                return jnp.maximum(m, scores(c).max(axis=0))

            m = lax.fori_loop(0, nt, pass1, jnp.full((8, 512), -jnp.inf, F32))
            m = jnp.broadcast_to(jnp.max(m, axis=0, keepdims=True), (8, 512))

            def pass2(c, carry):
                l, acc = carry
                p = jnp.exp2(scores(c) - m[None])
                pbf = p.reshape(128, 512).astype(BF)
                outs = []
                for j in range(4):
                    vj = _upk(vtb[pl.ds(pl.multiple_of(g * 64, 64) + j * 16, 16),
                                  pl.ds(pl.multiple_of(c * 128, 128), 128)])
                    outs.append(jnp.dot(vj, pbf[:, j * 128:(j + 1) * 128],
                                        preferred_element_type=F32))
                return l + p.sum(axis=0), acc + jnp.concatenate(outs, axis=1)

            l, acc = lax.fori_loop(0, nt, pass2,
                                   (jnp.zeros((8, 512), F32), jnp.zeros((DH, 512), F32)))
            lt = jnp.sum(l, axis=0, keepdims=True)
            o = acc * (1.0 / lt)
            st = jnp.concatenate([o[:, j * 128:(j + 1) * 128] for j in range(4)], axis=0)
            ob[pl.ds(pl.multiple_of(t * 128, 128), 128),
               pl.ds(pl.multiple_of(g * 128, 128), 128)] = st.T.astype(BF)
            return 0

        lax.fori_loop(0, (NH // 4) * nt, unit, 0)

    cp_bwo.wait()
    for qb in range(nqb):
        qs = slice(qb * QB, (qb + 1) * QB)
        res = jnp.dot(ob[qs, :], bwo[...], preferred_element_type=F32)
        stage[1, qs, :] = res.astype(BF)
        cp = pltpu.make_async_copy(stage.at[1, pl.ds(qb * QB, QB), :],
                                   out_h.at[pl.ds(qb * QB, QB), pl.ds(DM, DM)], osem.at[nqb + qb])
        cp.start()
        out_copies.append(cp)
    for cp in out_copies:
        cp.wait()


@jax.jit
def pallas_concat_heads__grouped_kv_mqa__sliding_block__prompt_kernel(
    A_x: jax.Array,
    A_wq: jax.Array,
    A_wk: jax.Array,
    A_wv: jax.Array,
    A_wo: jax.Array,
    B_x: jax.Array,
    B_wqkv: jax.Array,
    B_wo: jax.Array,
):
    any_spec = pl.BlockSpec(memory_space=pl.ANY)
    vm = pltpu.VMEM
    na = HPU * 128
    scratch = [
        vm((SEQ, DM), BF), vm((DM, DM), BF), vm((DM, DH), BF), vm((DM, DH), BF), vm((DM, DM), BF),
        vm((SEQ, DM), BF), vm((DM, 3 * DM), BF), vm((DM, DM), BF),
        vm((DM + 2 * DH, DM), BF), vm((DM // 2, SEQ), U32), vm((SEQ // 2, DH), U32),
        vm((DH // 2, SEQ), U32), vm((SEQ, DM), BF), vm((SEQ // CH, CH // 2, na), U32),
        vm((DH, na), F32), vm((8, na), F32),
        vm((2 * DM, DM), BF), vm((DM // 2, SEQ), U32), vm((NH // 4, SEQ // 2, 128), U32),
        vm((DM // 2, SEQ), U32), vm((SEQ, DM), BF), vm((2, 192, 512), U32),
        vm((DH, 512), F32), vm((8, 512), F32),
        vm((2, SEQ, DM), BF),
        pltpu.SemaphoreType.DMA((6 + 2 * (SEQ // QB),)),
        pltpu.SemaphoreType.DMA((2 * (SEQ // QB),)),
    ]
    out = pl.pallas_call(
        _kernel,
        out_shape=jax.ShapeDtypeStruct((SEQ, 2 * DM), BF),
        in_specs=[any_spec] * 8,
        out_specs=any_spec,
        scratch_shapes=scratch,
        compiler_params=pltpu.CompilerParams(vmem_limit_bytes=110 * 1024 * 1024),
        name="concat_heads_mqa_swa",
    )(A_x.reshape(SEQ, DM), A_wq, A_wk, A_wv, A_wo, B_x.reshape(SEQ, DM), B_wqkv, B_wo)
    return out.reshape(1, SEQ, 2 * DM)
```

```python
import functools

import jax
import jax.numpy as jnp
from jax import lax
import jax.experimental.pallas as pl
import jax.experimental.pallas.tpu as pltpu

SEQ = 2048
DM = 1024
HD = DM // 2
DH = 32
NH = 32
WIN = 256

BF = jnp.bfloat16
F32 = jnp.float32
U32 = jnp.uint32

LOG2E = 1.4426950408889634
QSCALE = (DH ** -0.5) * LOG2E
L_LO_BITS = (127 - 80) << 23
L_HI_BITS = (127 + 100) << 23
ONE_BITS = 127 << 23
INF_BITS = 255 << 23
NEG = -1.0e30

NT_DIMS = (((1,), (1,)), ((), ()))

HPU = 16
CH = 128
QB = 512
QBB = 1024
QBO = 512
SUMR = 16


def _pk(x):
    return pltpu.bitcast(x, U32)


def _upk(x):
    return pltpu.bitcast(x, BF)


class _Packed:
    def __init__(self, ref):
        self.ref = ref

    @staticmethod
    def _rows(rs):
        if isinstance(rs, slice):
            return slice(rs.start // 2, rs.stop // 2)
        return pl.ds(pl.multiple_of(rs.start // 2, 8), rs.size // 2)

    def __getitem__(self, idx):
        return _upk(self.ref[self._rows(idx[0]), idx[1]])

    def __setitem__(self, idx, v):
        self.ref[self._rows(idx[0]), idx[1]] = _pk(v)


def _nt(a, b):
    return lax.dot_general(a, b, NT_DIMS, preferred_element_type=F32)


def _nn(a, b):
    return jnp.dot(a, b, preferred_element_type=F32)


def _lhs_sums(blk, rows, dst):
    def job(r):
        a11, a12 = blk(0, 0, r).astype(F32), blk(0, 1, r).astype(F32)
        a21, a22 = blk(1, 0, r).astype(F32), blk(1, 1, r).astype(F32)
        for n, v in enumerate((a11 + a22, a21 + a22, a11 + a12, a21 - a11, a12 - a22)):
            dst[n, r // 2:(r + SUMR) // 2, :] = _pk(v.astype(BF))
    return [functools.partial(job, r) for r in range(0, rows, SUMR)]


def _rhs_sums(blk, rows, dst):
    def job(r):
        b11, b12 = blk(0, 0, r).astype(F32), blk(0, 1, r).astype(F32)
        b21, b22 = blk(1, 0, r).astype(F32), blk(1, 1, r).astype(F32)
        for n, v in enumerate((b11 + b22, b12 - b22, b21 - b11, b11 + b12, b21 + b22)):
            dst[n, r // 2:(r + SUMR) // 2, :] = _pk(v.astype(BF))
    return [functools.partial(job, r) for r in range(0, rows, SUMR)]


def _run(jobs):
    for job in jobs:
        job()


def _packed(sums):
    return lambda n, rs, cs: _upk(sums[n, rs.start // 2:rs.stop // 2, cs])


def _lhs_ops(sums, raw):
    put = _packed(sums)
    return [lambda rs, cs: put(0, rs, cs), lambda rs, cs: put(1, rs, cs),
            lambda rs, cs: raw(0, 0, rs, cs), lambda rs, cs: raw(1, 1, rs, cs),
            lambda rs, cs: put(2, rs, cs), lambda rs, cs: put(3, rs, cs),
            lambda rs, cs: put(4, rs, cs)]


def _rhs_ops(sums, raw):
    put = _packed(sums)
    return [lambda rs, cs: put(0, rs, cs), lambda rs, cs: raw(0, 0, rs, cs),
            lambda rs, cs: put(1, rs, cs), lambda rs, cs: put(2, rs, cs),
            lambda rs, cs: raw(1, 1, rs, cs), lambda rs, cs: put(3, rs, cs),
            lambda rs, cs: put(4, rs, cs)]


def _strassen(prod, fin, c, ntile, jobs):
    jobs = list(jobs)
    left = [7 * ntile]

    def side():
        n = -(-len(jobs) // left[0])
        left[0] -= 1
        for _ in range(n):
            jobs.pop(0)()

    for j in range(ntile):
        c[0] = prod(1, j)
        side()
        m = prod(3, j)
        fin(1, 0, j, c[0] + m)
        c[1] = m
        side()
        c[2] = prod(2, j)
        side()
        m = prod(4, j)
        fin(0, 1, j, c[2] + m)
        c[1] = c[1] - m
        side()
        m = prod(0, j)
        c[1] = c[1] + m
        c[3] = m - c[0] + c[2]
        side()
        fin(1, 1, j, c[3] + prod(5, j))
        side()
        fin(0, 0, j, c[1] + prod(6, j))
        side()
    assert not jobs


def _bits(x):
    return lax.bitcast_convert_type(x, jnp.int32)


def _fold(x, op):
    tiles = [x[r * 8:(r + 1) * 8, j * 128:(j + 1) * 128]
             for r in range(x.shape[0] // 8) for j in range(x.shape[1] // 128)]
    return functools.reduce(op, tiles)


def _watch_o(guard, o):
    lo, hi, top = guard
    return lo, hi, jnp.maximum(top, _fold(_bits(o) & 0x7FFFFFFF, jnp.maximum))


def _watch_l(guard, l):
    lo, hi, top = guard
    b = _bits(jnp.broadcast_to(l, (8, l.shape[1])))
    return (jnp.minimum(lo, _fold(b, jnp.minimum)), jnp.maximum(hi, _fold(b, jnp.maximum)), top)


def _new_guard():
    one = jnp.full((8, 128), ONE_BITS, jnp.int32)
    return one, one, jnp.zeros((8, 128), jnp.int32)


def _unsafe(guard):
    lo, hi, top = guard
    bad = jnp.logical_or(jnp.logical_or(lo < L_LO_BITS, hi > L_HI_BITS), top >= INF_BITS)
    return jnp.max(jnp.where(bad, 1.0, 0.0)) > 0.0


def _kernel(ax_h, awq_h, awkt_h, awvt_h, awo_h, bx_h, bwqkv_h, bwo_h, out_h,
            ax, awq, awo, bx, bwqkv, bwo,
            wkv, wta, woa_s, qta, ka, vta, oa, pa, accs, ls,
            wtb, wqb_s, wvb_s, wkb_s, wob_s, xb_s, qtb, kb, vtb, ob, bias, accb, lb,
            xo_s, cnn, cbt, stage, isem, osem):
    nqb = SEQ // QB
    nqbb = SEQ // QBB
    wta, wtb, oa, ob = _Packed(wta), _Packed(wtb), _Packed(oa), _Packed(ob)

    def rows(src, dst, r0, n, sem):
        return pltpu.make_async_copy(src.at[pl.ds(r0, n), :], dst.at[pl.ds(r0, n), :], sem)

    RB = 256
    nrb = DM // RB
    hq = QB // 2
    cp_awq = [pltpu.make_async_copy(awq_h.at[:, pl.ds(b * RB, RB)], awq.at[:, pl.ds(b * RB, RB)],
                                    isem.at[b]) for b in range(nrb)]
    cp_awk = pltpu.make_async_copy(awkt_h, wkv.at[pl.ds(DH, DH), :], isem.at[4])
    cp_awv = pltpu.make_async_copy(awvt_h, wkv.at[pl.ds(0, DH), :], isem.at[5])
    cp_awo = pltpu.make_async_copy(awo_h, awo, isem.at[6])
    cp_bw = pltpu.make_async_copy(bwqkv_h, bwqkv, isem.at[7])
    cp_bwo = pltpu.make_async_copy(bwo_h, bwo, isem.at[8])
    cp_ax = [rows(ax_h, ax, i * QB, QB, isem.at[10 + i]) for i in range(1, nqb)]
    cp_ax = [rows(ax_h, ax, hq, hq, isem.at[10])] + cp_ax
    cp_ax0 = rows(ax_h, ax, 0, hq, isem.at[9])
    cp_bx = [rows(bx_h, bx, i * QBB, QBB, isem.at[10 + nqb + i]) for i in range(nqbb)]

    for cp in ([cp_awq[0], cp_ax0, cp_ax[0]] + cp_awq[1:] + [cp_awv, cp_awk] + cp_ax[1:] + [cp_awo]):
        cp.start()

    def quad(ref, r0, c0, hr, hc):
        return lambda i, j, r: ref[r0 + i * hr + r:r0 + i * hr + r + SUMR, c0 + j * hc:c0 + (j + 1) * hc]

    def quad_t(ref, r0, c0, hr, hc):
        return lambda i, j, r: ref[r0 + j * hr + r:r0 + j * hr + r + SUMR, c0 + i * hc:c0 + (i + 1) * hc]

    def shift(sl, off):
        return slice(sl.start + off, sl.stop + off)

    def block(ref, r0, c0, hr, hc):
        return lambda i, j, rs, cs: ref[shift(rs, r0 + i * hr), shift(cs, c0 + j * hc)]

    def block_t(ref, r0, c0, hr, hc):
        return lambda i, j, rs, cs: ref[shift(rs, r0 + j * hr), shift(cs, c0 + i * hc)]

    def tile(j):
        return slice(j * 128, (j + 1) * 128)

    def prod_nt(a_ops, x_ops, h):
        return lambda n, j: _nt(a_ops[n](slice(0, HD), slice(0, HD)), x_ops[n](tile(j), slice(0, HD)))

    def prod_nn(a_ops, x_ops, h):
        return lambda n, j: _nn(x_ops[n](slice(0, h), slice(0, HD)), a_ops[n](slice(0, HD), tile(j)))

    def a_store_q(res, q0, nq, r0, nr):
        qta[r0 // 2:(r0 + nr) // 2, q0:q0 + nq] = _pk((res * QSCALE).astype(BF))

    def a_store(res, q0, r0):
        nr = res.shape[0]
        nq = min(max(DM - r0, 0), nr)
        if nq:
            qta[r0 // 2:(r0 + nq) // 2, q0:q0 + 128] = _pk((res[:nq] * QSCALE).astype(BF))
        if nq < nr:
            vta[:, q0:q0 + 128] = _pk(res[nq:nq + DH].astype(BF))
            ka[q0 // 2:(q0 + 128) // 2, :] = _pk(res[nq + DH:].T.astype(BF))

    def transposes(col0, row0):
        def job(b):
            wtb[row0 + b * 128:row0 + (b + 1) * 128, 0:DM] = bwqkv[:, col0 + b * 128:col0 + (b + 1) * 128].T
        return [functools.partial(job, b) for b in range(DM // 128)]

    def spread(pieces, jobs):
        jobs = list(jobs)
        for n, piece in enumerate(pieces):
            piece()
            _run([jobs.pop(0) for _ in range(-(-len(jobs) // (len(pieces) - n)))])
        assert not jobs

    def a_transpose(b):
        wta[b * RB:(b + 1) * RB, 0:DM] = awq[:, b * RB:(b + 1) * RB].T

    def a_first(b, q0=0, nq=QB):
        r1 = (b + 1) * RB if b + 1 < nrb else DM + 2 * DH
        res = _nt(wta[b * RB:r1, 0:DM], ax[q0:q0 + nq, :])
        for j in range(nq // 128):
            a_store(res[:, j * 128:(j + 1) * 128], q0 + j * 128, b * RB)

    cp_awq[0].wait()
    a_transpose(0)
    cp_ax0.wait()
    a_first(0, 0, hq)
    cp_ax[0].wait()
    a_first(0, hq, hq)
    cp_awq[1].wait()
    cp_awq[2].wait()
    a_transpose(1)
    a_first(1)
    a_transpose(2)
    cp_awq[3].wait()
    cp_awv.wait()
    cp_awk.wait()
    wta[DM:DM + 2 * DH, 0:DM] = wkv[...]
    a_first(2)
    a_transpose(3)
    a_first(3)

    def a_pieces(q0, nq, step):
        def piece(qq):
            res = _nt(wta[0:DM + 2 * DH, 0:DM], ax[qq:qq + step, :])
            for j in range(step // 128):
                a_store(res[:, j * 128:(j + 1) * 128], qq + j * 128, 0)
        return [functools.partial(piece, qq) for qq in range(q0, q0 + nq, step)]

    cp_ax[1].wait()
    spread(a_pieces(QB, QB, 512), [])
    cp_ax[2].wait()
    cp_ax[3].wait()
    cp_awo.wait()
    spread(a_pieces(2 * QB, 2 * QB, 256), _lhs_sums(quad_t(awo, 0, 0, HD, HD), HD, woa_s))

    na = HPU * 128
    noct = NH // HPU
    ncha = SEQ // CH

    def a_finalize(acc, l, u, bad):
        t = u // noct
        oc = u % noct
        lt = jnp.sum(l, axis=0, keepdims=True)
        o = acc * (1.0 / lt)
        bad = _watch_o(_watch_l(bad, lt), o)
        for g in range(HPU // 4):
            st = jnp.concatenate([o[:, (4 * g + j) * 128:(4 * g + j + 1) * 128] for j in range(4)],
                                 axis=0)
            col = pl.multiple_of(oc * (HPU * DH) + g * 128, 128)
            oa[pl.ds(pl.multiple_of(t * 128, 128), 128), pl.ds(col, 128)] = st.T.astype(BF)
        return bad

    def a_qt(u):
        t = u // noct
        oc = u % noct
        qall = qta[pl.ds(pl.multiple_of(oc * (HPU * DH // 2), HPU * DH // 2), HPU * DH // 2),
                   pl.ds(pl.multiple_of(t * 128, 128), 128)]
        return jnp.concatenate([_upk(qall[j * (DH // 2):(j + 1) * (DH // 2)]) for j in range(HPU)],
                               axis=1)

    def a_body(u, bad):
        qt = a_qt(u)
        l = jnp.zeros((8, na), F32)
        acc = jnp.zeros((DH, na), F32)
        bad = a_finalize(accs[...], ls[...], jnp.maximum(u - 1, 0), bad)
        for c in range(ncha + 1):
            if c < ncha:
                kc = _upk(ka[c * CH // 2:(c + 1) * CH // 2, :])
                p = jnp.exp2(jnp.dot(kc, qt, preferred_element_type=F32))
                l = l + p.reshape(CH // 8, 8, na).sum(axis=0)
                pa[c] = _pk(p.astype(BF))
            if c >= 1:
                vc = _upk(vta[:, (c - 1) * CH:c * CH])
                acc = acc + jnp.dot(vc, _upk(pa[c - 1]), preferred_element_type=F32)
        accs[...] = acc
        ls[...] = l
        return bad

    for cp in [cp_bw] + cp_bx + [cp_bwo]:
        cp.start()
    accs[...] = jnp.zeros((DH, na), F32)
    ls[...] = jnp.ones((8, na), F32)
    nunits = (SEQ // 128) * noct
    bad_a = lax.fori_loop(0, nunits, a_body, _new_guard())
    bad_a = a_finalize(accs[...], ls[...], nunits - 1, bad_a)
    for cp in [cp_bw] + cp_bx + [cp_bwo]:
        cp.wait()

    @pl.when(_unsafe(bad_a))
    def _a_fallback():
        def unit(u, _):
            qt = a_qt(u)

            def scores(c):
                kc = _upk(ka[pl.ds(pl.multiple_of(c * 64, 64), 64), :])
                return jnp.dot(kc, qt, preferred_element_type=F32).reshape(16, 8, na)

            def pass1(c, m):
                return jnp.maximum(m, scores(c).max(axis=0))

            m = lax.fori_loop(0, SEQ // 128, pass1, jnp.full((8, na), -jnp.inf, F32))
            m = jnp.broadcast_to(jnp.max(m, axis=0, keepdims=True), (8, na))

            def pass2(c, carry):
                l, acc = carry
                p = jnp.exp2(scores(c) - m[None])
                vc = _upk(vta[:, pl.ds(pl.multiple_of(c * 128, 128), 128)])
                acc = acc + jnp.dot(vc, p.reshape(128, na).astype(BF), preferred_element_type=F32)
                return l + p.sum(axis=0), acc

            l, acc = lax.fori_loop(0, SEQ // 128, pass2,
                                   (jnp.zeros((8, na), F32), jnp.zeros((DH, na), F32)))
            a_finalize(acc, l, u, _new_guard())
            return 0

        lax.fori_loop(0, nunits, unit, 0)

    out_copies = []
    ho = QBO // 2

    def out_proj(o_ref, w_ref, w_s, half, jobs_of):
        _run(_rhs_sums(quad_t(o_ref, 0, 0, ho, HD), ho, xo_s.at[0]))
        for qb in range(SEQ // QBO):
            q0 = qb * QBO
            a_ops = _lhs_ops(w_s, block_t(w_ref, 0, 0, HD, HD))
            b_ops = _rhs_ops(xo_s.at[qb % 2], block_t(o_ref, q0, 0, ho, HD))
            jobs = jobs_of(qb)
            if qb + 1 < SEQ // QBO:
                jobs = _rhs_sums(quad_t(o_ref, q0 + QBO, 0, ho, HD), ho, xo_s.at[(qb + 1) % 2]) + jobs
            last = half == 1 and qb + 1 == SEQ // QBO

            def send(r0, nr, c0, nc):
                cp = pltpu.make_async_copy(
                    stage.at[half, pl.ds(r0, nr), pl.ds(c0, nc)],
                    out_h.at[pl.ds(r0, nr), pl.ds(half * DM + c0, nc)], osem.at[len(out_copies)])
                cp.start()
                out_copies.append(cp)

            def fin(i, k, j, v):
                r0 = q0 + k * ho
                stage[half, r0:r0 + ho, i * HD + j * 128:i * HD + (j + 1) * 128] = v.astype(BF)
                if last and j == HD // 128 - 1:
                    send(r0, ho, i * HD, HD)

            _strassen(prod_nn(a_ops, b_ops, ho), fin, cnn, HD // 128, jobs)
            if not last:
                send(q0, QBO, 0, DM)

    def b_weight_work(qb):
        if qb == 0:
            return transposes(0, 0) + _lhs_sums(quad(wtb, 0, 0, HD, HD), HD, wqb_s)
        if qb == 1:
            return transposes(2 * DM, DM) + _lhs_sums(quad(wtb, DM, 0, HD, HD), HD, wvb_s)
        if qb == 2:
            return _lhs_sums(quad_t(bwqkv, 0, DM, HD, HD), HD, wkb_s)
        return (_rhs_sums(quad_t(bx, 0, 0, QBB // 2, HD), QBB // 2, xb_s.at[0])
                + _lhs_sums(quad_t(bwo, 0, 0, HD, HD), HD, wob_s)[:16])

    out_proj(oa, awo, woa_s, 0, b_weight_work)

    hb = QBB // 2
    for qb in range(nqbb):
        q0 = qb * QBB
        b_ops = _rhs_ops(xb_s.at[qb % 2], block_t(bx, q0, 0, hb, HD))

        def fin_q(i, k, j, v):
            c0 = q0 + k * hb + j * 128
            qtb[i * HD // 2:(i + 1) * HD // 2, c0:c0 + 128] = _pk((v * QSCALE).astype(BF))

        def fin_v(i, k, j, v):
            c0 = q0 + k * hb + j * 128
            vtb[i * HD // 2:(i + 1) * HD // 2, c0:c0 + 128] = _pk(v.astype(BF))

        def fin_k(i, k, j, v):
            r0 = (q0 + k * hb) // 2
            kb[i * 4 + j, r0:r0 + hb // 2, :] = _pk(v.astype(BF))

        if qb + 1 < nqbb:
            jobs = _rhs_sums(quad_t(bx, q0 + QBB, 0, hb, HD), hb, xb_s.at[(qb + 1) % 2])
        else:
            jobs = _lhs_sums(quad_t(bwo, 0, 0, HD, HD), HD, wob_s)[16:]
        n3 = len(jobs) // 3
        a_ops = _lhs_ops(wqb_s, block(wtb, 0, 0, HD, HD))
        _strassen(prod_nt(a_ops, b_ops, hb), fin_q, cbt, hb // 128, jobs[:n3])
        a_ops = _lhs_ops(wvb_s, block(wtb, DM, 0, HD, HD))
        _strassen(prod_nt(a_ops, b_ops, hb), fin_v, cbt, hb // 128, jobs[n3:2 * n3])
        a_ops = _lhs_ops(wkb_s, block_t(bwqkv, 0, DM, HD, HD))
        _strassen(prod_nn(a_ops, b_ops, hb), fin_k, cbt, HD // 128, jobs[2 * n3:])

    nt = SEQ // 128

    def lanes(shape):
        return lax.broadcasted_iota(jnp.int32, shape, 1)

    row32 = lax.broadcasted_iota(jnp.int32, (32, 128), 0)
    qq32 = lanes((32, 128)) % 32
    bias[0] = jnp.where(row32 <= qq32, 0.0, NEG)
    bias[1] = jnp.where(row32 > qq32, 0.0, NEG)

    def even(shape):
        return (lanes(shape) // 32) % 2 == 0

    def low(shape):
        return lanes(shape) < 64

    def xperm(x, h):
        if h == 0:
            return x
        if h == 2:
            return pltpu.roll(x, 64, 1)
        if h == 1:
            return jnp.where(even(x.shape), pltpu.roll(x, 96, 1), pltpu.roll(x, 32, 1))
        return jnp.where(even(x.shape), pltpu.roll(x, 32, 1), pltpu.roll(x, 96, 1))

    ev8, lo8 = even((8, 128)), low((8, 128))

    def sel(m, a, b):
        if a is None and b is None:
            return None
        shape = (a if a is not None else b).shape
        if shape[0] < 8:
            return jnp.where(m[0:1], a, b)
        split = (shape[0] // 8, 8, 128)
        a = 0.0 if a is None else a.reshape(split)
        b = 0.0 if b is None else b.reshape(split)
        return jnp.where(m[None], a, b).reshape(shape)

    def butterfly(src, shape):
        ev, lo = ev8, lo8
        e0, e1 = sel(ev, src[0], src[1]), sel(ev, src[1], src[0])
        e2, e3 = sel(ev, src[2], src[3]), sel(ev, src[3], src[2])
        return [sel(lo, e0, e2), sel(lo, e1, e3), sel(lo, e2, e0), sel(lo, e3, e1)]

    def b_store(o4, g, t0):
        st = jnp.concatenate(o4, axis=0)
        ob[t0:t0 + 128, pl.ds(pl.multiple_of(g * 128, 128), 128)] = st.T.astype(BF)

    def b_finalize(acc, r, g, t, bad):
        o = acc * r[0:1, :]
        bad = _watch_o(bad, o)
        b_store([xperm(o[:, h * 128:(h + 1) * 128], h) for h in range(4)], g, t * 128)
        return bad

    def b_body(g, bad):
        v0 = pl.multiple_of(g * 64, 64)
        lg16 = lanes((16, 128)) // 32

        def qk(t, bad):
            q4 = qtb[pl.ds(v0, 64), t * 128:(t + 1) * 128]
            rr = [xperm(q4[h * 16:(h + 1) * 16], h) for h in range(4)]
            ws = [_upk(jnp.concatenate([jnp.where(lg16 == (i ^ h), rr[h], 0) for h in range(4)],
                                       axis=0)) for i in range(4)]
            d0, d1 = max(4 * t - 8, 0), 4 * t + 4
            mid = [s for s in range(d0, d1) if 4 * t - 4 <= s < 4 * t]
            edge = [s for s in range(d0, d1) if s not in mid]
            dest = {}
            ls_ = [None] * 4
            for grp in (mid, edge):
                src = {}
                for i in range(4):
                    ss = [s for s in grp if max(4 * t + i - 8, 0) <= s <= 4 * t + i]
                    if not ss:
                        continue
                    kc = _upk(jnp.concatenate([kb[g, s * 16:(s + 1) * 16, :] for s in ss], axis=0))
                    sc = jnp.dot(kc, ws[i], preferred_element_type=F32)
                    for n, s in enumerate(ss):
                        ps = sc[n * 32:(n + 1) * 32]
                        if s == 4 * t + i:
                            ps = ps + bias[0]
                        elif s == 4 * t + i - 8:
                            ps = ps + bias[1]
                        ps = jnp.exp2(ps)
                        part = ps.reshape(4, 8, 128).sum(axis=0)
                        ls_[i] = part if ls_[i] is None else ls_[i] + part
                        src[(i, s)] = ps
                for s in grp:
                    dest[s] = butterfly([src.get((i, s)) for i in range(4)], (32, 128))
            lt = [jnp.sum(l, axis=0, keepdims=True) for l in ls_]
            bad = _watch_l(bad, jnp.concatenate(lt, axis=1))
            r = jnp.concatenate(butterfly([1.0 / l for l in lt], (1, 128)), axis=1)
            ps = [jnp.concatenate([dest[s][h] for s in range(d0, d1)], axis=0).astype(BF)
                  for h in range(4)]
            return ps, r, bad

        def pv(t, ps):
            d0, d1 = max(4 * t - 8, 0), 4 * t + 4
            return jnp.concatenate(
                [jnp.dot(_upk(vtb[pl.ds(v0 + h * 16, 16), d0 * 32:d1 * 32]), ps[h],
                         preferred_element_type=F32) for h in range(4)], axis=1)

        bad = b_finalize(accb[...], lb[...], jnp.maximum(g - 1, 0), nt - 1, bad)
        prev = acc_prev = r_pp = None
        for t in range(nt + 1):
            cur = None
            if t < nt:
                ps, r, bad = qk(t, bad)
                cur = (ps, r)
            if t >= 2:
                bad = b_finalize(acc_prev, r_pp, g, t - 2, bad)
            if t >= 1:
                acc_prev = pv(t - 1, prev[0])
                r_pp = prev[1]
            prev = cur
        accb[...] = acc_prev
        lb[...] = jnp.broadcast_to(r_pp, (8, 512))
        return bad

    accb[...] = jnp.zeros((DH, 512), F32)
    lb[...] = jnp.ones((8, 512), F32)
    bad_b = lax.fori_loop(0, NH // 4, b_body, _new_guard())
    bad_b = b_finalize(accb[...], lb[...], NH // 4 - 1, nt - 1, bad_b)

    @pl.when(_unsafe(bad_b))
    def _b_fallback():
        fill = -999292928.0 * LOG2E

        row = lax.broadcasted_iota(jnp.int32, (128, 128), 0)
        colq = lax.broadcasted_iota(jnp.int32, (128, 128), 1)

        def tile4(m):
            return jnp.concatenate([m, m, m, m], axis=1)

        def unit(u, _):
            g = u // nt
            t = u % nt
            q4 = qtb[pl.ds(pl.multiple_of(g * 64, 64), 64), pl.ds(pl.multiple_of(t * 128, 128), 128)]
            z = jnp.zeros((16, 128), U32)
            w = _upk(jnp.concatenate(
                [jnp.concatenate([q4[j * 16:(j + 1) * 16] if i == j else z for i in range(4)], axis=0)
                 for j in range(4)], axis=1))

            def scores(c):
                kc = _upk(kb[g, pl.ds(pl.multiple_of(c * 64, 64), 64), :])
                s = jnp.dot(kc, w, preferred_element_type=F32)
                d = (colq + t * 128) - (row + c * 128)
                valid = tile4(jnp.logical_and(d >= 0, d < WIN))
                return jnp.where(valid, s, fill).reshape(16, 8, 512)

            def pass1(c, m):
                return jnp.maximum(m, scores(c).max(axis=0))

            m = lax.fori_loop(0, nt, pass1, jnp.full((8, 512), -jnp.inf, F32))
            m = jnp.broadcast_to(jnp.max(m, axis=0, keepdims=True), (8, 512))

            def pass2(c, carry):
                l, acc = carry
                p = jnp.exp2(scores(c) - m[None])
                pbf = p.reshape(128, 512).astype(BF)
                outs = []
                for j in range(4):
                    vj = _upk(vtb[pl.ds(pl.multiple_of(g * 64, 64) + j * 16, 16),
                                  pl.ds(pl.multiple_of(c * 128, 128), 128)])
                    outs.append(jnp.dot(vj, pbf[:, j * 128:(j + 1) * 128],
                                        preferred_element_type=F32))
                return l + p.sum(axis=0), acc + jnp.concatenate(outs, axis=1)

            l, acc = lax.fori_loop(0, nt, pass2,
                                   (jnp.zeros((8, 512), F32), jnp.zeros((DH, 512), F32)))
            lt = jnp.sum(l, axis=0, keepdims=True)
            o = acc * (1.0 / lt)
            st = jnp.concatenate([o[:, j * 128:(j + 1) * 128] for j in range(4)], axis=0)
            ob[pl.ds(pl.multiple_of(t * 128, 128), 128),
               pl.ds(pl.multiple_of(g * 128, 128), 128)] = st.T.astype(BF)
            return 0

        lax.fori_loop(0, (NH // 4) * nt, unit, 0)

    out_proj(ob, bwo, wob_s, 1, lambda qb: [])
    for cp in out_copies:
        cp.wait()


@jax.jit
def pallas_concat_heads__grouped_kv_mqa__sliding_block__prompt_kernel(
    A_x: jax.Array,
    A_wq: jax.Array,
    A_wk: jax.Array,
    A_wv: jax.Array,
    A_wo: jax.Array,
    B_x: jax.Array,
    B_wqkv: jax.Array,
    B_wo: jax.Array,
):
    any_spec = pl.BlockSpec(memory_space=pl.ANY)
    vm = pltpu.VMEM
    na = HPU * 128
    w_sums = vm((5, HD // 2, HD), U32)
    scratch = [
        vm((SEQ, DM), BF), vm((DM, DM), BF), vm((DM, DM), BF),
        vm((SEQ, DM), BF), vm((DM, 3 * DM), BF), vm((DM, DM), BF),
        vm((2 * DH, DM), BF), vm((DM // 2 + DH, DM), U32), w_sums,
        vm((DM // 2, SEQ), U32), vm((SEQ // 2, DH), U32),
        vm((DH // 2, SEQ), U32), vm((SEQ // 2, DM), U32), vm((SEQ // CH, CH // 2, na), U32),
        vm((DH, na), F32), vm((8, na), F32),
        vm((DM, DM), U32), w_sums, w_sums, w_sums, w_sums, vm((2, 5, QBB // 4, HD), U32),
        vm((DM // 2, SEQ), U32), vm((NH // 4, SEQ // 2, 128), U32),
        vm((DM // 2, SEQ), U32), vm((SEQ // 2, DM), U32), vm((2, 32, 128), F32),
        vm((DH, 512), F32), vm((8, 512), F32),
        vm((2, 5, QBO // 4, HD), U32),
        vm((4, QBO // 2, 128), F32), vm((4, HD, 128), F32),
        vm((2, SEQ, DM), BF),
        pltpu.SemaphoreType.DMA((16,)),
        pltpu.SemaphoreType.DMA((16,)),
    ]
    out = pl.pallas_call(
        _kernel,
        out_shape=jax.ShapeDtypeStruct((SEQ, 2 * DM), BF),
        in_specs=[any_spec] * 8,
        out_specs=any_spec,
        scratch_shapes=scratch,
        compiler_params=pltpu.CompilerParams(vmem_limit_bytes=120 * 1024 * 1024),
        name="concat_heads_mqa_swa",
    )(A_x.reshape(SEQ, DM), A_wq, A_wk.T, A_wv.T, A_wo, B_x.reshape(SEQ, DM), B_wqkv, B_wo)
    return out.reshape(1, SEQ, 2 * DM)
```

```python
import functools

import jax
import jax.numpy as jnp
from jax import lax
import jax.experimental.pallas as pl
import jax.experimental.pallas.tpu as pltpu

SEQ = 2048
DM = 1024
HD = DM // 2
DH = 32
NH = 32
WIN = 256

BF = jnp.bfloat16
F32 = jnp.float32
U32 = jnp.uint32

LOG2E = 1.4426950408889634
QSCALE = (DH ** -0.5) * LOG2E
L_LO_BITS = (127 - 80) << 23
L_HI_BITS = (127 + 124) << 23
ONE_BITS = 127 << 23
INF_BITS = 255 << 23
NEG = -1.0e30

NT_DIMS = (((1,), (1,)), ((), ()))

HPU = 16
CH = 128
QB = 512
QBB = 1024
A_BLOCKS = (512, 512, 512, 512)
B_BLOCKS = (512, 1024, 512)
QBO = max(A_BLOCKS + B_BLOCKS)
SUMR = 16


def _pk(x):
    return pltpu.bitcast(x, U32)


def _upk(x):
    return pltpu.bitcast(x, BF)


class _Packed:
    def __init__(self, ref):
        self.ref = ref

    @staticmethod
    def _rows(rs):
        if isinstance(rs, slice):
            return slice(rs.start // 2, rs.stop // 2)
        return pl.ds(pl.multiple_of(rs.start // 2, 8), rs.size // 2)

    def __getitem__(self, idx):
        return _upk(self.ref[self._rows(idx[0]), idx[1]])

    def __setitem__(self, idx, v):
        self.ref[self._rows(idx[0]), idx[1]] = _pk(v)


def _nt(a, b):
    return lax.dot_general(a, b, NT_DIMS, preferred_element_type=F32)


def _nn(a, b):
    return jnp.dot(a, b, preferred_element_type=F32)


def _sum_jobs(blk, rows, dst, combine):
    def job(r):
        quads = [blk(i, j, r).astype(F32) for i in (0, 1) for j in (0, 1)]
        for n, v in enumerate(combine(*quads)):
            dst[n, r // 2:(r + SUMR) // 2, :] = _pk(v.astype(BF))
    return [functools.partial(job, r) for r in range(0, rows, SUMR)]


def _lhs_sums(blk, rows, dst):
    return _sum_jobs(blk, rows, dst, lambda a11, a12, a21, a22: (
        a11 + a22, a21 + a22, a11 + a12, a21 - a11, a12 - a22))


def _rhs_sums(blk, rows, dst):
    return _sum_jobs(blk, rows, dst, lambda b11, b12, b21, b22: (
        b11 + b22, b12 - b22, b21 - b11, b11 + b12, b21 + b22))


def _run(jobs):
    for job in jobs:
        job()


def _packed(sums):
    return lambda n, rs, cs: _upk(sums[n, rs.start // 2:rs.stop // 2, cs])


def _lhs_ops(sums, raw):
    put = _packed(sums)
    return [lambda rs, cs: put(0, rs, cs), lambda rs, cs: put(1, rs, cs),
            lambda rs, cs: raw(0, 0, rs, cs), lambda rs, cs: raw(1, 1, rs, cs),
            lambda rs, cs: put(2, rs, cs), lambda rs, cs: put(3, rs, cs),
            lambda rs, cs: put(4, rs, cs)]


def _rhs_ops(sums, raw):
    put = _packed(sums)
    return [lambda rs, cs: put(0, rs, cs), lambda rs, cs: raw(0, 0, rs, cs),
            lambda rs, cs: put(1, rs, cs), lambda rs, cs: put(2, rs, cs),
            lambda rs, cs: raw(1, 1, rs, cs), lambda rs, cs: put(3, rs, cs),
            lambda rs, cs: put(4, rs, cs)]


def _strassen(prod, fin, c, ntile, jobs):
    jobs = list(jobs)
    left = [7 * ntile]

    def side():
        n = -(-len(jobs) // left[0])
        left[0] -= 1
        for _ in range(n):
            jobs.pop(0)()

    for j in range(ntile):
        c[0] = prod(1, j)
        side()
        m = prod(3, j)
        fin(1, 0, j, c[0] + m)
        c[1] = m
        side()
        c[2] = prod(2, j)
        side()
        m = prod(4, j)
        fin(0, 1, j, c[2] + m)
        c[1] = c[1] - m
        side()
        m = prod(0, j)
        c[1] = c[1] + m
        c[3] = m - c[0] + c[2]
        side()
        fin(1, 1, j, c[3] + prod(5, j))
        side()
        fin(0, 0, j, c[1] + prod(6, j))
        side()
    assert not jobs


def _bits(x):
    return lax.bitcast_convert_type(x, jnp.int32)


def _fold(x, op):
    tiles = [x[r * 8:(r + 1) * 8, j * 128:(j + 1) * 128]
             for r in range(x.shape[0] // 8) for j in range(x.shape[1] // 128)]
    return functools.reduce(op, tiles)


def _watch_o(guard, o):
    lo, hi, top = guard
    return lo, hi, jnp.maximum(top, _fold(_bits(o) & 0x7FFFFFFF, jnp.maximum))


def _watch_l(guard, l):
    lo, hi, top = guard
    b = _bits(jnp.broadcast_to(l, (8, l.shape[1])))
    return (jnp.minimum(lo, _fold(b, jnp.minimum)), jnp.maximum(hi, _fold(b, jnp.maximum)), top)


def _new_guard():
    one = jnp.full((8, 128), ONE_BITS, jnp.int32)
    return one, one, jnp.zeros((8, 128), jnp.int32)


def _unsafe(guard):
    lo, hi, top = guard
    bad = jnp.logical_or(jnp.logical_or(lo < L_LO_BITS, hi > L_HI_BITS), top >= INF_BITS)
    return jnp.max(jnp.where(bad, 1.0, 0.0)) > 0.0


def _kernel(ax_h, awq_h, awkt_h, awvt_h, awo_h, bx_h, bwqkv_h, bwo_h, out_h,
            ax, awq, awo, bx, bwqkv, bwo,
            wkv, wta, woa_s, qta, ka, vta, oa, pa, accs, ls,
            wtb, wqb_s, wvb_s, wkb_s, wob_s, xb_s, qtb, kb, vtb, ob, bias, accb, lb,
            xo_s, cnn, cbt, stage, isem, osem):
    nqb = SEQ // QB
    nqbb = SEQ // QBB
    wta, wtb, oa, ob = _Packed(wta), _Packed(wtb), _Packed(oa), _Packed(ob)

    def rows(src, dst, r0, n, sem):
        return pltpu.make_async_copy(src.at[pl.ds(r0, n), :], dst.at[pl.ds(r0, n), :], sem)

    RB = 256
    nrb = DM // RB
    hq = QB // 2
    cp_awq = [pltpu.make_async_copy(awq_h.at[:, pl.ds(b * RB, RB)], awq.at[:, pl.ds(b * RB, RB)],
                                    isem.at[b]) for b in range(nrb)]
    cp_awk = pltpu.make_async_copy(awkt_h, wkv.at[pl.ds(DH, DH), :], isem.at[4])
    cp_awv = pltpu.make_async_copy(awvt_h, wkv.at[pl.ds(0, DH), :], isem.at[5])
    cp_awo = pltpu.make_async_copy(awo_h, awo, isem.at[6])
    cp_bw = pltpu.make_async_copy(bwqkv_h, bwqkv, isem.at[7])
    cp_bwo = pltpu.make_async_copy(bwo_h, bwo, isem.at[8])
    cp_ax = [rows(ax_h, ax, i * QB, QB, isem.at[10 + i]) for i in range(1, nqb)]
    cp_ax = [rows(ax_h, ax, hq, hq, isem.at[10])] + cp_ax
    cp_ax0 = rows(ax_h, ax, 0, hq, isem.at[9])
    cp_bx = [rows(bx_h, bx, i * QBB, QBB, isem.at[10 + nqb + i]) for i in range(nqbb)]

    for cp in ([cp_awq[0], cp_ax0, cp_ax[0]] + cp_awq[1:] + [cp_awv, cp_awk] + cp_ax[1:] + [cp_awo]):
        cp.start()

    def quad(ref, r0, c0, hr, hc):
        return lambda i, j, r: ref[r0 + i * hr + r:r0 + i * hr + r + SUMR,
                                   c0 + j * hc:c0 + (j + 1) * hc]

    def quad_t(ref, r0, c0, hr, hc):
        return lambda i, j, r: ref[r0 + j * hr + r:r0 + j * hr + r + SUMR,
                                   c0 + i * hc:c0 + (i + 1) * hc]

    def shift(sl, off):
        return slice(sl.start + off, sl.stop + off)

    def block(ref, r0, c0, hr, hc):
        return lambda i, j, rs, cs: ref[shift(rs, r0 + i * hr), shift(cs, c0 + j * hc)]

    def block_t(ref, r0, c0, hr, hc):
        return lambda i, j, rs, cs: ref[shift(rs, r0 + j * hr), shift(cs, c0 + i * hc)]

    def tile(j):
        return slice(j * 128, (j + 1) * 128)

    def prod_nt(a_ops, x_ops):
        return lambda n, j: _nt(a_ops[n](slice(0, HD), slice(0, HD)), x_ops[n](tile(j), slice(0, HD)))

    def prod_nn(a_ops, x_ops, h):
        return lambda n, j: _nn(x_ops[n](slice(0, h), slice(0, HD)), a_ops[n](slice(0, HD), tile(j)))

    def a_store(res, q0, r0):
        nr = res.shape[0]
        nq = min(max(DM - r0, 0), nr)
        if nq:
            qta[r0 // 2:(r0 + nq) // 2, q0:q0 + 128] = _pk((res[:nq] * QSCALE).astype(BF))
        if nq < nr:
            vta[:, q0:q0 + 128] = _pk(res[nq:nq + DH].astype(BF))
            ka[q0 // 2:(q0 + 128) // 2, :] = _pk(res[nq + DH:].T.astype(BF))

    def transposes(col0, row0):
        def job(b):
            cols = bwqkv[:, col0 + b * 128:col0 + (b + 1) * 128]
            wtb[row0 + b * 128:row0 + (b + 1) * 128, 0:DM] = cols.T
        return [functools.partial(job, b) for b in range(DM // 128)]

    def spread(pieces, jobs):
        jobs = list(jobs)
        for n, piece in enumerate(pieces):
            piece()
            _run([jobs.pop(0) for _ in range(-(-len(jobs) // (len(pieces) - n)))])
        assert not jobs

    def a_transpose(b):
        wta[b * RB:(b + 1) * RB, 0:DM] = awq[:, b * RB:(b + 1) * RB].T

    def a_first(b, q0=0, nq=QB):
        r1 = (b + 1) * RB if b + 1 < nrb else DM + 2 * DH
        res = _nt(wta[b * RB:r1, 0:DM], ax[q0:q0 + nq, :])
        for j in range(nq // 128):
            a_store(res[:, j * 128:(j + 1) * 128], q0 + j * 128, b * RB)

    cp_awq[0].wait()
    a_transpose(0)
    cp_ax0.wait()
    a_first(0, 0, hq)
    cp_ax[0].wait()
    a_first(0, hq, hq)
    cp_awq[1].wait()
    cp_awq[2].wait()
    a_transpose(1)
    a_first(1)
    a_transpose(2)
    cp_awq[3].wait()
    cp_awv.wait()
    cp_awk.wait()
    wta[DM:DM + 2 * DH, 0:DM] = wkv[...]
    a_first(2)
    a_transpose(3)
    a_first(3)

    def a_pieces(q0, nq, step):
        def piece(qq):
            res = _nt(wta[0:DM + 2 * DH, 0:DM], ax[qq:qq + step, :])
            for j in range(step // 128):
                a_store(res[:, j * 128:(j + 1) * 128], qq + j * 128, 0)
        return [functools.partial(piece, qq) for qq in range(q0, q0 + nq, step)]

    cp_ax[1].wait()
    spread(a_pieces(QB, QB, 512), [])
    cp_ax[2].wait()
    cp_ax[3].wait()
    cp_awo.wait()
    spread(a_pieces(2 * QB, 2 * QB, 256), _lhs_sums(quad_t(awo, 0, 0, HD, HD), HD, woa_s))

    na = HPU * 128
    noct = NH // HPU
    ncha = SEQ // CH

    def a_finalize(acc, l, u, guard):
        t = u // noct
        oc = u % noct
        lt = jnp.sum(l, axis=0, keepdims=True)
        o = acc * (1.0 / lt)
        guard = _watch_o(_watch_l(guard, lt), o)
        for g in range(HPU // 4):
            st = jnp.concatenate([o[:, (4 * g + j) * 128:(4 * g + j + 1) * 128] for j in range(4)],
                                 axis=0)
            col = pl.multiple_of(oc * (HPU * DH) + g * 128, 128)
            oa[pl.ds(pl.multiple_of(t * 128, 128), 128), pl.ds(col, 128)] = st.T.astype(BF)
        return guard

    def a_qt(u):
        t = u // noct
        oc = u % noct
        qall = qta[pl.ds(pl.multiple_of(oc * (HPU * DH // 2), HPU * DH // 2), HPU * DH // 2),
                   pl.ds(pl.multiple_of(t * 128, 128), 128)]
        return jnp.concatenate([_upk(qall[j * (DH // 2):(j + 1) * (DH // 2)]) for j in range(HPU)],
                               axis=1)

    def a_body(u, guard):
        qt = a_qt(u)
        l = jnp.zeros((8, na), F32)
        acc = jnp.zeros((DH, na), F32)
        guard = a_finalize(accs[...], ls[...], jnp.maximum(u - 1, 0), guard)
        for c in range(ncha + 1):
            if c < ncha:
                kc = _upk(ka[c * CH // 2:(c + 1) * CH // 2, :])
                p = jnp.exp2(jnp.dot(kc, qt, preferred_element_type=F32))
                l = l + p.reshape(CH // 8, 8, na).sum(axis=0)
                pa[c] = _pk(p.astype(BF))
            if c >= 1:
                vc = _upk(vta[:, (c - 1) * CH:c * CH])
                acc = acc + jnp.dot(vc, _upk(pa[c - 1]), preferred_element_type=F32)
        accs[...] = acc
        ls[...] = l
        return guard

    for cp in [cp_bw] + cp_bx + [cp_bwo]:
        cp.start()
    accs[...] = jnp.zeros((DH, na), F32)
    ls[...] = jnp.ones((8, na), F32)
    nunits = (SEQ // 128) * noct
    guard_a = lax.fori_loop(0, nunits, a_body, _new_guard())
    guard_a = a_finalize(accs[...], ls[...], nunits - 1, guard_a)
    for cp in [cp_bw] + cp_bx + [cp_bwo]:
        cp.wait()

    @pl.when(_unsafe(guard_a))
    def _a_fallback():
        def unit(u, _):
            qt = a_qt(u)

            def scores(c):
                kc = _upk(ka[pl.ds(pl.multiple_of(c * 64, 64), 64), :])
                return jnp.dot(kc, qt, preferred_element_type=F32).reshape(16, 8, na)

            def pass1(c, m):
                return jnp.maximum(m, scores(c).max(axis=0))

            m = lax.fori_loop(0, SEQ // 128, pass1, jnp.full((8, na), -jnp.inf, F32))
            m = jnp.broadcast_to(jnp.max(m, axis=0, keepdims=True), (8, na))

            def pass2(c, carry):
                l, acc = carry
                p = jnp.exp2(scores(c) - m[None])
                vc = _upk(vta[:, pl.ds(pl.multiple_of(c * 128, 128), 128)])
                acc = acc + jnp.dot(vc, p.reshape(128, na).astype(BF), preferred_element_type=F32)
                return l + p.sum(axis=0), acc

            l, acc = lax.fori_loop(0, SEQ // 128, pass2,
                                   (jnp.zeros((8, na), F32), jnp.zeros((DH, na), F32)))
            a_finalize(acc, l, u, _new_guard())
            return 0

        lax.fori_loop(0, nunits, unit, 0)

    out_copies = []

    def out_proj(o_ref, w_ref, w_s, half, blocks, jobs_of):
        def o_sums(n, q0):
            return _rhs_sums(quad_t(o_ref, q0, 0, blocks[n] // 2, HD), blocks[n] // 2, xo_s.at[n % 2])

        _run(o_sums(0, 0))
        q0 = 0
        for qb, nq in enumerate(blocks):
            ho = nq // 2
            a_ops = _lhs_ops(w_s, block_t(w_ref, 0, 0, HD, HD))
            b_ops = _rhs_ops(xo_s.at[qb % 2], block_t(o_ref, q0, 0, ho, HD))
            jobs = jobs_of(qb)
            if qb + 1 < len(blocks):
                jobs = o_sums(qb + 1, q0 + nq) + jobs
            last = half == 1 and qb + 1 == len(blocks)

            def send(r0, nr, c0, nc):
                cp = pltpu.make_async_copy(
                    stage.at[half, pl.ds(r0, nr), pl.ds(c0, nc)],
                    out_h.at[pl.ds(r0, nr), pl.ds(half * DM + c0, nc)], osem.at[len(out_copies)])
                cp.start()
                out_copies.append(cp)

            def fin(i, k, j, v):
                r0 = q0 + k * ho
                stage[half, r0:r0 + ho, i * HD + j * 128:i * HD + (j + 1) * 128] = v.astype(BF)
                if last and j == HD // 128 - 1:
                    send(r0, ho, i * HD, HD)

            _strassen(prod_nn(a_ops, b_ops, ho), fin, cnn.at[:, pl.ds(0, ho), :], HD // 128, jobs)
            if not last:
                send(q0, nq, 0, DM)
            q0 += nq

    wq_jobs = transposes(0, 0) + _lhs_sums(quad(wtb, 0, 0, HD, HD), HD, wqb_s)
    wv_jobs = transposes(2 * DM, DM) + _lhs_sums(quad(wtb, DM, 0, HD, HD), HD, wvb_s)
    wk_jobs = _lhs_sums(quad_t(bwqkv, 0, DM, HD, HD), HD, wkb_s)
    wo_jobs = _lhs_sums(quad_t(bwo, 0, 0, HD, HD), HD, wob_s)
    x0_jobs = _rhs_sums(quad_t(bx, 0, 0, QBB // 2, HD), QBB // 2, xb_s.at[0])
    x1_jobs = _rhs_sums(quad_t(bx, QBB, 0, QBB // 2, HD), QBB // 2, xb_s.at[1])
    early = wq_jobs + x0_jobs

    def b_weight_work(qb):
        cut = (0, 14, 28, 42, len(early))
        return early[cut[qb]:cut[qb + 1]]

    out_proj(oa, awo, woa_s, 0, A_BLOCKS, b_weight_work)

    hb = QBB // 2
    for qb in range(nqbb):
        q0 = qb * QBB
        b_ops = _rhs_ops(xb_s.at[qb % 2], block_t(bx, q0, 0, hb, HD))

        def fin_q(i, k, j, v):
            c0 = q0 + k * hb + j * 128
            qtb[i * HD // 2:(i + 1) * HD // 2, c0:c0 + 128] = _pk((v * QSCALE).astype(BF))

        def fin_v(i, k, j, v):
            c0 = q0 + k * hb + j * 128
            vtb[i * HD // 2:(i + 1) * HD // 2, c0:c0 + 128] = _pk(v.astype(BF))

        def fin_k(i, k, j, v):
            r0 = (q0 + k * hb) // 2
            kb[i * 4 + j, r0:r0 + hb // 2, :] = _pk(v.astype(BF))

        jobs = ((wv_jobs, wk_jobs, x1_jobs), (wo_jobs[:11], wo_jobs[11:22], wo_jobs[22:]))[qb]
        a_ops = _lhs_ops(wqb_s, block(wtb, 0, 0, HD, HD))
        _strassen(prod_nt(a_ops, b_ops), fin_q, cbt, hb // 128, jobs[0])
        a_ops = _lhs_ops(wvb_s, block(wtb, DM, 0, HD, HD))
        _strassen(prod_nt(a_ops, b_ops), fin_v, cbt, hb // 128, jobs[1])
        a_ops = _lhs_ops(wkb_s, block_t(bwqkv, 0, DM, HD, HD))
        _strassen(prod_nn(a_ops, b_ops, hb), fin_k, cbt, HD // 128, jobs[2])

    nt = SEQ // 128

    def lanes(shape):
        return lax.broadcasted_iota(jnp.int32, shape, 1)

    row32 = lax.broadcasted_iota(jnp.int32, (32, 128), 0)
    qq32 = lanes((32, 128)) % 32
    bias[0] = jnp.where(row32 <= qq32, 0.0, NEG)
    bias[1] = jnp.where(row32 > qq32, 0.0, NEG)

    def even(shape):
        return (lanes(shape) // 32) % 2 == 0

    def low(shape):
        return lanes(shape) < 64

    def xperm(x, h):
        if h == 0:
            return x
        if h == 2:
            return pltpu.roll(x, 64, 1)
        if h == 1:
            return jnp.where(even(x.shape), pltpu.roll(x, 96, 1), pltpu.roll(x, 32, 1))
        return jnp.where(even(x.shape), pltpu.roll(x, 32, 1), pltpu.roll(x, 96, 1))

    ev8, lo8 = even((8, 128)), low((8, 128))

    def sel(m, a, b):
        if a is None and b is None:
            return None
        shape = (a if a is not None else b).shape
        if shape[0] < 8:
            return jnp.where(m[0:1], a, b)
        split = (shape[0] // 8, 8, 128)
        a = 0.0 if a is None else a.reshape(split)
        b = 0.0 if b is None else b.reshape(split)
        return jnp.where(m[None], a, b).reshape(shape)

    def butterfly(src):
        e0, e1 = sel(ev8, src[0], src[1]), sel(ev8, src[1], src[0])
        e2, e3 = sel(ev8, src[2], src[3]), sel(ev8, src[3], src[2])
        return [sel(lo8, e0, e2), sel(lo8, e1, e3), sel(lo8, e2, e0), sel(lo8, e3, e1)]

    def b_store(o4, g, t0):
        st = jnp.concatenate(o4, axis=0)
        ob[t0:t0 + 128, pl.ds(pl.multiple_of(g * 128, 128), 128)] = st.T.astype(BF)

    def b_finalize(acc, r, g, t, guard):
        o = acc * r[0:1, :]
        guard = _watch_o(guard, o)
        b_store([xperm(o[:, h * 128:(h + 1) * 128], h) for h in range(4)], g, t * 128)
        return guard

    def b_body(g, guard):
        v0 = pl.multiple_of(g * 64, 64)
        lg16 = lanes((16, 128)) // 32

        def qk(t, guard):
            q4 = qtb[pl.ds(v0, 64), t * 128:(t + 1) * 128]
            rr = [xperm(q4[h * 16:(h + 1) * 16], h) for h in range(4)]
            ws = [_upk(jnp.concatenate([jnp.where(lg16 == (i ^ h), rr[h], 0) for h in range(4)],
                                       axis=0)) for i in range(4)]
            d0, d1 = max(4 * t - 8, 0), 4 * t + 4
            mid = [s for s in range(d0, d1) if 4 * t - 4 <= s < 4 * t]
            edge = [s for s in range(d0, d1) if s not in mid]
            dest = {}
            ls_ = [None] * 4
            for grp in (mid, edge):
                src = {}
                for i in range(4):
                    ss = [s for s in grp if max(4 * t + i - 8, 0) <= s <= 4 * t + i]
                    if not ss:
                        continue
                    kc = _upk(jnp.concatenate([kb[g, s * 16:(s + 1) * 16, :] for s in ss], axis=0))
                    sc = jnp.dot(kc, ws[i], preferred_element_type=F32)
                    for n, s in enumerate(ss):
                        ps = sc[n * 32:(n + 1) * 32]
                        if s == 4 * t + i:
                            ps = ps + bias[0]
                        elif s == 4 * t + i - 8:
                            ps = ps + bias[1]
                        ps = jnp.exp2(ps)
                        part = ps.reshape(4, 8, 128).sum(axis=0)
                        ls_[i] = part if ls_[i] is None else ls_[i] + part
                        src[(i, s)] = ps
                for s in grp:
                    dest[s] = butterfly([src.get((i, s)) for i in range(4)])
            lt = [jnp.sum(l, axis=0, keepdims=True) for l in ls_]
            guard = _watch_l(guard, jnp.concatenate(lt, axis=1))
            r = jnp.concatenate(butterfly([1.0 / l for l in lt]), axis=1)
            ps = [jnp.concatenate([dest[s][h] for s in range(d0, d1)], axis=0).astype(BF)
                  for h in range(4)]
            return ps, r, guard

        def pv(t, ps):
            d0, d1 = max(4 * t - 8, 0), 4 * t + 4
            return jnp.concatenate(
                [jnp.dot(_upk(vtb[pl.ds(v0 + h * 16, 16), d0 * 32:d1 * 32]), ps[h],
                         preferred_element_type=F32) for h in range(4)], axis=1)

        guard = b_finalize(accb[...], lb[...], jnp.maximum(g - 1, 0), nt - 1, guard)
        prev = acc_prev = r_pp = None
        for t in range(nt + 1):
            cur = None
            if t < nt:
                ps, r, guard = qk(t, guard)
                cur = (ps, r)
            if t >= 2:
                guard = b_finalize(acc_prev, r_pp, g, t - 2, guard)
            if t >= 1:
                acc_prev = pv(t - 1, prev[0])
                r_pp = prev[1]
            prev = cur
        accb[...] = acc_prev
        lb[...] = jnp.broadcast_to(r_pp, (8, 512))
        return guard

    accb[...] = jnp.zeros((DH, 512), F32)
    lb[...] = jnp.ones((8, 512), F32)
    def b_four(v, guard):
        for i in range(4):
            guard = b_body(4 * v + i, guard)
        return guard

    guard_b = lax.fori_loop(0, NH // 16, b_four, _new_guard())
    guard_b = b_finalize(accb[...], lb[...], NH // 4 - 1, nt - 1, guard_b)

    @pl.when(_unsafe(guard_b))
    def _b_fallback():
        fill = -999292928.0 * LOG2E

        row = lax.broadcasted_iota(jnp.int32, (128, 128), 0)
        colq = lax.broadcasted_iota(jnp.int32, (128, 128), 1)

        def tile4(m):
            return jnp.concatenate([m, m, m, m], axis=1)

        def unit(u, _):
            g = u // nt
            t = u % nt
            q4 = qtb[pl.ds(pl.multiple_of(g * 64, 64), 64), pl.ds(pl.multiple_of(t * 128, 128), 128)]
            z = jnp.zeros((16, 128), U32)
            w = _upk(jnp.concatenate(
                [jnp.concatenate([q4[j * 16:(j + 1) * 16] if i == j else z for i in range(4)], axis=0)
                 for j in range(4)], axis=1))

            def scores(c):
                kc = _upk(kb[g, pl.ds(pl.multiple_of(c * 64, 64), 64), :])
                s = jnp.dot(kc, w, preferred_element_type=F32)
                d = (colq + t * 128) - (row + c * 128)
                valid = tile4(jnp.logical_and(d >= 0, d < WIN))
                return jnp.where(valid, s, fill).reshape(16, 8, 512)

            def pass1(c, m):
                return jnp.maximum(m, scores(c).max(axis=0))

            m = lax.fori_loop(0, nt, pass1, jnp.full((8, 512), -jnp.inf, F32))
            m = jnp.broadcast_to(jnp.max(m, axis=0, keepdims=True), (8, 512))

            def pass2(c, carry):
                l, acc = carry
                p = jnp.exp2(scores(c) - m[None])
                pbf = p.reshape(128, 512).astype(BF)
                outs = []
                for j in range(4):
                    vj = _upk(vtb[pl.ds(pl.multiple_of(g * 64, 64) + j * 16, 16),
                                  pl.ds(pl.multiple_of(c * 128, 128), 128)])
                    outs.append(jnp.dot(vj, pbf[:, j * 128:(j + 1) * 128],
                                        preferred_element_type=F32))
                return l + p.sum(axis=0), acc + jnp.concatenate(outs, axis=1)

            l, acc = lax.fori_loop(0, nt, pass2,
                                   (jnp.zeros((8, 512), F32), jnp.zeros((DH, 512), F32)))
            lt = jnp.sum(l, axis=0, keepdims=True)
            o = acc * (1.0 / lt)
            st = jnp.concatenate([o[:, j * 128:(j + 1) * 128] for j in range(4)], axis=0)
            ob[pl.ds(pl.multiple_of(t * 128, 128), 128),
               pl.ds(pl.multiple_of(g * 128, 128), 128)] = st.T.astype(BF)
            return 0

        lax.fori_loop(0, (NH // 4) * nt, unit, 0)

    out_proj(ob, bwo, wob_s, 1, B_BLOCKS, lambda qb: [])
    for cp in out_copies:
        cp.wait()


@jax.jit
def pallas_concat_heads__grouped_kv_mqa__sliding_block__prompt_kernel(
    A_x: jax.Array,
    A_wq: jax.Array,
    A_wk: jax.Array,
    A_wv: jax.Array,
    A_wo: jax.Array,
    B_x: jax.Array,
    B_wqkv: jax.Array,
    B_wo: jax.Array,
):
    any_spec = pl.BlockSpec(memory_space=pl.ANY)
    vm = pltpu.VMEM
    na = HPU * 128
    w_sums = vm((5, HD // 2, HD), U32)
    scratch = [
        vm((SEQ, DM), BF), vm((DM, DM), BF), vm((DM, DM), BF),
        vm((SEQ, DM), BF), vm((DM, 3 * DM), BF), vm((DM, DM), BF),
        vm((2 * DH, DM), BF), vm((DM // 2 + DH, DM), U32), w_sums,
        vm((DM // 2, SEQ), U32), vm((SEQ // 2, DH), U32),
        vm((DH // 2, SEQ), U32), vm((SEQ // 2, DM), U32), vm((SEQ // CH, CH // 2, na), U32),
        vm((DH, na), F32), vm((8, na), F32),
        vm((DM, DM), U32), w_sums, w_sums, w_sums, w_sums, vm((2, 5, QBB // 4, HD), U32),
        vm((DM // 2, SEQ), U32), vm((NH // 4, SEQ // 2, 128), U32),
        vm((DM // 2, SEQ), U32), vm((SEQ // 2, DM), U32), vm((2, 32, 128), F32),
        vm((DH, 512), F32), vm((8, 512), F32),
        vm((2, 5, QBO // 4, HD), U32),
        vm((4, QBO // 2, 128), F32), vm((4, HD, 128), F32),
        vm((2, SEQ, DM), BF),
        pltpu.SemaphoreType.DMA((16,)),
        pltpu.SemaphoreType.DMA((16,)),
    ]
    out = pl.pallas_call(
        _kernel,
        out_shape=jax.ShapeDtypeStruct((SEQ, 2 * DM), BF),
        in_specs=[any_spec] * 8,
        out_specs=any_spec,
        scratch_shapes=scratch,
        compiler_params=pltpu.CompilerParams(vmem_limit_bytes=120 * 1024 * 1024),
        name="concat_heads_mqa_swa",
    )(A_x.reshape(SEQ, DM), A_wq, A_wk.T, A_wv.T, A_wo, B_x.reshape(SEQ, DM), B_wqkv, B_wo)
    return out.reshape(1, SEQ, 2 * DM)
```
